```python
import os as _os
_os.environ.setdefault("JAX_PLATFORMS", "cpu")
import jax
import jax.numpy as jnp

def _softmax(x, axis=-1):
    return jax.nn.softmax(x, axis=axis)
def _gelu(x):
    return jax.nn.gelu(x, approximate=True)
def _silu(x):
    return jax.nn.silu(x)
def _sigmoid(x):
    return jax.nn.sigmoid(x)
def _layernorm(x, axis=-1, eps=1e-5):
    m = jnp.mean(x, axis=axis, keepdims=True)
    v = jnp.var(x, axis=axis, keepdims=True)
    return (x - m) / jnp.sqrt(v + eps)
def _scatter_add(tgt, idx, src, axis=0):
    return tgt.at[idx].add(src)
def _segment_sum(src, seg, n):
    return jax.ops.segment_sum(src, seg, n)
class _Rng:
    def __init__(self, key):
        self._k = key
    def _next(self):
        self._k, sub = jax.random.split(self._k)
        return sub
    def normal(self, shape):
        return jax.random.normal(self._next(), shape, dtype=jnp.bfloat16)
    def randint(self, lo, hi, shape):
        return jax.random.randint(self._next(), shape, lo, hi, dtype=jnp.int32)
    def uniform(self, shape, lo=0.0, hi=1.0):
        return jax.random.uniform(self._next(), shape, jnp.bfloat16, lo, hi)
    def permutation(self, n):
        return jax.random.permutation(self._next(), n)


kernel_name = 'gated_mix__sliding_block__dense_activation_silu__prompt'

def setup_inputs():
    _rng = _Rng(jax.random.key(int.from_bytes(__import__("os").urandom(4), "little")))
    _w = (lambda a: (lambda t: t.astype(jnp.bfloat16) if jnp.issubdtype(t.dtype, jnp.floating) else t)(jnp.asarray(a)))
    def _A_setup():
        B, S, D = 1, 2048, 640
        return {
            "x": _w((lambda *s: _rng.normal(s) * 0.05)(B, S, D)),
            "wqkv": _w((lambda *s: _rng.normal(s) * 0.4)(D, 3 * D)),
            "wo": _w((lambda *s: _rng.normal(s) * 0.05)(D, D)),
        }
    _A_in = _A_setup()

    def _B_setup():
        B, S, D, F = 1, 2048, 640, 1536
        return {
            "x": _w((lambda *s: _rng.normal(s) * 0.05)(B, S, D)),
            "w1": _w((lambda *s: _rng.normal(s) * 1.6)(D, F) * (D ** -0.5)),
            "w2": _w((lambda *s: _rng.normal(s) * 1.6)(F, D) * (F ** -0.5)),
        }
    _B_in = _B_setup()

    return {
        "A_x": _A_in["x"],
        "A_wqkv": _A_in["wqkv"],
        "A_wo": _A_in["wo"],
        "B_x": _B_in["x"],
        "B_w1": _B_in["w1"],
        "B_w2": _B_in["w2"],
        "gate_w": _w((lambda *s: _rng.normal(s) * 0.05)(640) * 16.0),
    }

def reference(A_x, A_wqkv, A_wo, B_x, B_w1, B_w2, gate_w):
    def _A_ref(x, wqkv, wo):
        B, S, D = x.shape
        H = 32; Dh = D // H; W = 256
        qkv = (lambda x, *d: x.transpose(*d))((x @ wqkv).reshape(B, S, 3, H, Dh), 2, 0, 3, 1, 4)
        q, k, v = qkv[0], qkv[1], qkv[2]
        scores = jnp.einsum("bhqd,bhkd->bhqk", q, k) * (Dh ** -0.5)
        idx = jnp.arange(S)
        mask = (idx[:, None] - idx[None, :] >= 0) & (idx[:, None] - idx[None, :] < W)
        scores = jnp.where(mask[None, None], scores, -1e9)
        p = _softmax(scores, axis=-1)
        o = jnp.einsum("bhqk,bhkd->bhqd", p, v)
        return (lambda x, *d: x.transpose(*d))(o, 0, 2, 1, 3).reshape(B, S, D) @ wo

    def _B_ref(x, w1, w2):
        h = jnp.einsum("bsd,df->bsf", x, w1)
        h = _silu(h)
        out = jnp.einsum("bsf,fd->bsd", h, w2)
        return out

    x = A_x
    g = _sigmoid((x * gate_w).sum(-1, keepdims=True))
    a = _A_ref(x, A_wqkv, A_wo)
    b = _B_ref(x, B_w1, B_w2)
    return g * a + (1 - g) * b
```

```python
import jax
import jax.numpy as jnp
from jax import lax
import jax.experimental.pallas as pl
import jax.experimental.pallas.tpu as pltpu

S, D, F = 2048, 640, 1536
H, DH, WIN = 32, 20, 256
NQ = 8
NT = S // 128
XB = 256
PB = 512

bf16 = jnp.bfloat16
f32 = jnp.float32
i32 = jnp.int32

LOG2E = 1.4426950408889634
QSCALE = float(DH ** -0.5) * LOG2E
NEG = -1e30


def _bc32(x):
    return pltpu.bitcast(x, i32)


def _bc16(x):
    return pltpu.bitcast(x, bf16)


def _dot(a, b):
    return jnp.dot(a, b, preferred_element_type=f32)


def _kernel(x_hbm, wqkv_hbm, wo_hbm, w1_hbm, w2_hbm, gw_hbm, out_hbm,
            x_v, wqkv_v, wo_v, w1_v, w2_v, gw_v,
            wqvT_v, qm_v, k4_v, vt_v, ot_v, mask_v, bias_v, sa_v, sb_v,
            out_v, sems, osems):
    nxb = S // XB

    def x_copy(j):
        return pltpu.make_async_copy(x_hbm.at[pl.ds(j * XB, XB), :],
                                     x_v.at[pl.ds(j * XB, XB), :], sems.at[j])

    def wqkv_copy(part):
        return pltpu.make_async_copy(wqkv_hbm.at[:, pl.ds(part * D, D)],
                                     wqkv_v.at[:, pl.ds(part * D, D)], sems.at[nxb + part])

    w1_copy = pltpu.make_async_copy(w1_hbm, w1_v, sems.at[nxb + 3])
    w2_copy = pltpu.make_async_copy(w2_hbm, w2_v, sems.at[nxb + 4])
    wo_copy = pltpu.make_async_copy(wo_hbm, wo_v, sems.at[nxb + 5])
    gw_copy = pltpu.make_async_copy(gw_hbm, gw_v, sems.at[nxb + 6])

    x_copy(0).start()
    wqkv_copy(1).start()
    for j in range(1, 4):
        x_copy(j).start()
    wqkv_copy(0).start()
    wqkv_copy(2).start()
    for j in range(4, nxb):
        x_copy(j).start()
    w1_copy.start()
    w2_copy.start()
    wo_copy.start()
    gw_copy.start()

    row = lax.broadcasted_iota(i32, (80, 128), 0)
    lane = lax.broadcasted_iota(i32, (80, 128), 1)
    for i in range(2):
        for r in range(2):
            ha = (row >= 40 * i) & (row < 40 * i + 20)
            hb = (row >= 40 * i + 20) & (row < 40 * i + 40)
            lo = lane < 64
            m = (ha & (lo if r == 0 else ~lo)) | (hb & (~lo if r == 0 else lo))
            w = _bc32(jnp.where(m, 1.0, 0.0).astype(bf16))
            mask_v[2 * i + r] = (jnp.where((w & 0xFFFF) != 0, 0xFFFF, 0)
                                 | jnp.where((w >> 16) != 0, jnp.int32(-65536), 0))
    row = lax.broadcasted_iota(i32, (64, 128), 0)
    lm = lax.broadcasted_iota(i32, (64, 128), 1) & 63
    bias_v[0] = jnp.where(row > lm, 0.0, NEG).astype(f32)
    bias_v[1] = jnp.where(row <= lm, 0.0, NEG).astype(f32)

    def k_proj(j, _):
        for jj in range(PB // XB):
            x_copy(j * (PB // XB) + jj).wait()
        t0 = pl.multiple_of(j * PB, PB)
        kb = _bc32(_dot(x_v[pl.ds(t0, PB), :], wqkv_v[:, D:2 * D]).astype(bf16))
        lane_k = lax.broadcasted_iota(i32, (PB // 2, 128), 1)
        for c in range(NQ):
            o, t = (80 * c) % 128, (80 * c) // 128
            tile = kb[:, t * 128:(t + 1) * 128]
            if o + 80 > 128:
                tile = jnp.where(lane_k >= o, tile, kb[:, (t + 1) * 128:(t + 2) * 128])
            if o:
                tile = pltpu.roll(tile, 128 - o, 1)
            k4_v[pl.ds(pl.multiple_of(j * (PB // 2), PB // 2), PB // 2), c * 128:(c + 1) * 128] = tile

    wqkv_copy(1).wait()
    lax.fori_loop(0, S // PB, k_proj, None)

    wqkv_copy(0).wait()
    wqkv_copy(2).wait()
    for t in range(D // 128):
        wqvT_v[0:D, t * 128:(t + 1) * 128] = wqkv_v[t * 128:(t + 1) * 128, 0:D].T
        wqvT_v[D:2 * D, t * 128:(t + 1) * 128] = wqkv_v[t * 128:(t + 1) * 128, 2 * D:3 * D].T

    def qv_proj(j, _):
        rowq = lax.broadcasted_iota(i32, (40, 128), 0)
        odd = jnp.broadcast_to((rowq >= 20)[None], (H // 2, 40, 128)).reshape(D, 128)
        for t in range(PB // 128):
            tt = j * (PB // 128) + t
            xb = x_v[pl.ds(pl.multiple_of(tt * 128, 128), 128), :]
            qv = lax.dot_general(wqvT_v[...], xb, (((1,), (1,)), ((), ())),
                                 preferred_element_type=f32)
            q = qv[:D] * QSCALE
            q = jnp.where(odd, pltpu.roll(q, 64, 1), q)
            qm_v[:, pl.ds(pl.multiple_of(tt * 128, 128), 128)] = _bc32(q.astype(bf16))
            v = jnp.concatenate([qv[D:].reshape(H // 2, 40, 128),
                                 jnp.ones((H // 2, 8, 128), f32)], axis=1)
            vt_v[tt] = _bc32(v.reshape(H // 2 * 48, 128).astype(bf16))

    lax.fori_loop(0, S // PB, qv_proj, None)

    units = [(0, 0), (0, 1), (1, 0), (1, 1)]

    def qk_unit(c, T, i, r, nprev):
        lo = 16 * i
        qq = qm_v[pl.ds(pl.multiple_of(c * 40 + lo, 8), 24), pl.ds(pl.multiple_of(T * 128, 128), 128)]
        w = qq & mask_v[2 * i + r, lo:lo + 24]
        w = _bc16(jnp.concatenate(([jnp.zeros((lo, 128), i32)] if lo else [])
                                  + [w, jnp.zeros((64 - 24 - lo, 128), i32)], axis=0))
        if nprev == 2:
            krow, nrow = pl.multiple_of((T - 2) * 64 + 32 * r, 32), 160
        else:
            krow, nrow = 0, 64 * nprev + 32 * (r + 1)
        kk = _bc16(k4_v[pl.ds(krow, nrow), pl.ds(pl.multiple_of(c * 128, 128), 128)])
        return _dot(kk, w)

    def softmax_unit(s, r, nprev):
        n = s.shape[0]
        parts = []
        if nprev == 2:
            parts.append(s[0:64] + bias_v[0])
            parts.append(s[64:n - 64])
        elif n > 64:
            parts.append(s[0:n - 64])
        parts.append(s[n - 64:n] + bias_v[1])
        m = jnp.max(parts[0], axis=0, keepdims=True)
        for p in parts[1:]:
            m = jnp.maximum(m, jnp.max(p, axis=0, keepdims=True))
        ps = [jnp.exp2(p - m) for p in parts]
        z = jnp.zeros((64, 128), f32)
        if r == 0:
            ps = ps + [z]
        elif nprev == 2:
            ps = [z] + ps
        return jnp.concatenate(ps, axis=0).astype(bf16)

    def pv_unit(c, T, i, pf, nprev):
        prow = pl.multiple_of((c * 2 + i) * 24, 8)
        vv = jnp.concatenate([_bc16(vt_v[T - nprev + j, pl.ds(prow, 24), :])
                              for j in range(nprev + 1)], axis=1)
        R = _dot(vv, pf)
        return (R[:40].reshape(5, 8, 128) * (1.0 / R[40:48])[None]).reshape(40, 128)

    def finish(c, T, Rs):
        lane_o = lax.broadcasted_iota(i32, (40, 128), 1)
        row_o = lax.broadcasted_iota(i32, (40, 128), 0)
        outs = []
        for i in range(2):
            R0, R1 = Rs[2 * i], Rs[2 * i + 1]
            A = jnp.where(lane_o < 64, R0, R1)
            B = pltpu.roll(jnp.where(lane_o < 64, R1, R0), 64, 1)
            outs.append(jnp.where(row_o < 20, A, B))
        o = jnp.concatenate(outs, axis=0).astype(bf16)
        ot_v[pl.ds(pl.multiple_of(c * 40, 8), 40), pl.ds(pl.multiple_of(T * 128, 128), 128)] = _bc32(o)

    def edge(c, _):
        for T in range(2):
            Rs = []
            for (i, r) in units:
                pf = softmax_unit(qk_unit(c, T, i, r, T), r, T)
                Rs.append(pv_unit(c, T, i, pf, T))
            finish(c, T, Rs)

    lax.fori_loop(0, NQ, edge, None)

    def ct(idx):
        return idx % NQ, idx // NQ + 2

    def qk_group(idx, s_ref):
        c, T = ct(idx)
        for u, (i, r) in enumerate(units):
            s_ref[u] = qk_unit(c, T, i, r, 2)

    def step(idx, cur_ref, nxt_ref, do_qk):
        c, T = ct(idx)
        Rs = []
        for u, (i, r) in enumerate(units):
            if do_qk:
                cn, Tn = ct(idx + 1)
                nxt_ref[u] = qk_unit(cn, Tn, i, r, 2)
            Rs.append(pv_unit(c, T, i, softmax_unit(cur_ref[u], r, 2), 2))
        finish(c, T, Rs)

    ngroups = (NT - 2) * NQ
    NSTEP = 4
    qk_group(0, sa_v)

    def attn_body(it, _):
        for k in range(NSTEP // 2):
            step(NSTEP * it + 2 * k, sa_v, sb_v, True)
            step(NSTEP * it + 2 * k + 1, sb_v, sa_v, True)

    lax.fori_loop(0, ngroups // NSTEP - 1, attn_body, None)
    base = ngroups - NSTEP
    for k in range(NSTEP // 2):
        step(base + 2 * k, sa_v, sb_v, True)
        step(base + 2 * k + 1, sb_v, sa_v, k < NSTEP // 2 - 1)

    w1_copy.wait()
    w2_copy.wait()
    wo_copy.wait()
    gw_copy.wait()
    gw = gw_v[...].astype(f32).reshape(1, D)

    def out_copy(j, slot):
        return pltpu.make_async_copy(out_v.at[slot], out_hbm.at[pl.ds(pl.multiple_of(j * XB, XB), XB), :],
                                     osems.at[slot])

    def final(j, _):
        slot = j % 2
        t0 = pl.multiple_of(j * XB, XB)
        xb = x_v[pl.ds(t0, XB), :]
        h = _dot(xb, w1_v[...])
        h = (h * jax.nn.sigmoid(h)).astype(bf16)
        b = _dot(h, w2_v[...])
        oT = _bc16(ot_v[:, pl.ds(t0, XB)])
        a = lax.dot_general(oT, wo_v[...], (((0,), (0,)), ((), ())), preferred_element_type=f32)
        g = jax.nn.sigmoid(jnp.sum(xb.astype(f32) * gw, axis=1, keepdims=True))

        @pl.when(j >= 2)
        def _():
            out_copy(j - 2, slot).wait()

        out_v[slot] = (g * a + (1.0 - g) * b).astype(bf16)
        out_copy(j, slot).start()

    lax.fori_loop(0, nxb, final, None)
    out_copy(nxb - 2, 0).wait()
    out_copy(nxb - 1, 1).wait()


@jax.jit
def pallas_gated_mix__sliding_block__dense_activation_silu__prompt_kernel(
    A_x: jax.Array,
    A_wqkv: jax.Array,
    A_wo: jax.Array,
    B_x: jax.Array,
    B_w1: jax.Array,
    B_w2: jax.Array,
    gate_w: jax.Array,
):
    del B_x
    any_spec = pl.BlockSpec(memory_space=pl.ANY)
    out = pl.pallas_call(
        _kernel,
        out_shape=jax.ShapeDtypeStruct((S, D), bf16),
        in_specs=[any_spec] * 6,
        out_specs=any_spec,
        scratch_shapes=[
            pltpu.VMEM((S, D), bf16),
            pltpu.VMEM((D, 3 * D), bf16),
            pltpu.VMEM((D, D), bf16),
            pltpu.VMEM((D, F), bf16),
            pltpu.VMEM((F, D), bf16),
            pltpu.VMEM((D,), bf16),
            pltpu.VMEM((2 * D, D), bf16),
            pltpu.VMEM((D // 2, S), i32),
            pltpu.VMEM((S // 2, NQ * 128), i32),
            pltpu.VMEM((NT, H // 2 * 24, 128), i32),
            pltpu.VMEM((D // 2, S), i32),
            pltpu.VMEM((4, 40, 128), i32),
            pltpu.VMEM((2, 64, 128), f32),
            pltpu.VMEM((4, 320, 128), f32),
            pltpu.VMEM((4, 320, 128), f32),
            pltpu.VMEM((2, XB, D), bf16),
            pltpu.SemaphoreType.DMA((S // XB + 7,)),
            pltpu.SemaphoreType.DMA((2,)),
        ],
        compiler_params=pltpu.CompilerParams(vmem_limit_bytes=100 * 1024 * 1024),
    )(A_x.reshape(S, D), A_wqkv, A_wo, B_w1, B_w2, gate_w)
    return out.reshape(1, S, D)
```

```python
import jax
import jax.numpy as jnp
from jax import lax
import jax.experimental.pallas as pl
import jax.experimental.pallas.tpu as pltpu

S, D, F = 2048, 640, 1536
H, DH = 32, 20
NQ = 8
NT = S // 128
XB = 256
PB = 512

bf16 = jnp.bfloat16
f32 = jnp.float32
i32 = jnp.int32

LOG2E = 1.4426950408889634
QSCALE = float(DH ** -0.5) * LOG2E
NEG = -1e30


def _bc32(x):
    return pltpu.bitcast(x, i32)


def _bc16(x):
    return pltpu.bitcast(x, bf16)


def _dot(a, b):
    return jnp.dot(a, b, preferred_element_type=f32)


def _kernel(x_hbm, wqkv_hbm, wo_hbm, w1_hbm, w2_hbm, gw_hbm, out_hbm,
            x_v, wqkv_v, wo_v, w1_v, w2_v, gw_v,
            wqvT_v, kn_v, qm_v, k4_v, vt_v, ot_v, mask_v, bias_v, sa_v, sb_v,
            out_v, sems, osems):
    nxb = S // XB

    def x_copy(j):
        return pltpu.make_async_copy(x_hbm.at[pl.ds(j * XB, XB), :],
                                     x_v.at[pl.ds(j * XB, XB), :], sems.at[j])

    def wqkv_copy(part):
        return pltpu.make_async_copy(wqkv_hbm.at[:, pl.ds(part * D, D)],
                                     wqkv_v.at[:, pl.ds(part * D, D)], sems.at[nxb + part])

    w1_copy = pltpu.make_async_copy(w1_hbm, w1_v, sems.at[nxb + 3])
    w2_copy = pltpu.make_async_copy(w2_hbm, w2_v, sems.at[nxb + 4])
    wo_copy = pltpu.make_async_copy(wo_hbm, wo_v, sems.at[nxb + 5])
    gw_copy = pltpu.make_async_copy(gw_hbm, gw_v, sems.at[nxb + 6])

    x_copy(0).start()
    wqkv_copy(1).start()
    for j in range(1, nxb):
        x_copy(j).start()
    wqkv_copy(0).start()
    wqkv_copy(2).start()
    w1_copy.start()
    w2_copy.start()
    wo_copy.start()
    gw_copy.start()

    row = lax.broadcasted_iota(i32, (80, 128), 0)
    lane = lax.broadcasted_iota(i32, (80, 128), 1)
    for i in range(2):
        for r in range(2):
            ha = (row >= 40 * i) & (row < 40 * i + 20)
            hb = (row >= 40 * i + 20) & (row < 40 * i + 40)
            lo = lane < 64
            m = (ha & (lo if r == 0 else ~lo)) | (hb & (~lo if r == 0 else lo))
            w = _bc32(jnp.where(m, 1.0, 0.0).astype(bf16))
            mask_v[2 * i + r] = (jnp.where((w & 0xFFFF) != 0, 0xFFFF, 0)
                                 | jnp.where((w >> 16) != 0, jnp.int32(-65536), 0))
    row = lax.broadcasted_iota(i32, (64, 128), 0)
    lm = lax.broadcasted_iota(i32, (64, 128), 1) & 63
    bias_v[0] = jnp.where(row > lm, 0.0, NEG).astype(f32)
    bias_v[1] = jnp.where(row <= lm, 0.0, NEG).astype(f32)

    def k_rows(t0, n):
        t0 = pl.multiple_of(t0, XB)
        kb = _bc32(_dot(x_v[pl.ds(t0, n), :], wqkv_v[:, D:2 * D]).astype(bf16))
        kn_v[pl.ds(pl.multiple_of(t0 // 2, XB // 2), n // 2), :] = kb

    def k_wait(j):
        for jj in range(PB // XB):
            x_copy(j * (PB // XB) + jj).wait()

    def k_proj(j, _, wait=True):
        if wait:
            k_wait(j)
        k_rows(j * PB, PB)

    wqkv_copy(1).wait()
    for jj in range(PB // XB):
        x_copy(jj).wait()
        k_rows(jj * XB, XB)
    lax.fori_loop(1, S // PB - 1, k_proj, None)
    k_wait(S // PB - 1)

    wqkv_copy(0).wait()
    wqkv_copy(2).wait()
    k_proj(S // PB - 1, None, wait=False)
    for t in range(D // 128):
        wqvT_v[0:D, t * 128:(t + 1) * 128] = wqkv_v[t * 128:(t + 1) * 128, 0:D].T
        wqvT_v[D:2 * D, t * 128:(t + 1) * 128] = wqkv_v[t * 128:(t + 1) * 128, 2 * D:3 * D].T

    def qv_proj(j, _):
        kb = kn_v[pl.ds(pl.multiple_of(j * (PB // 2), PB // 2), PB // 2), :]
        lane_k = lax.broadcasted_iota(i32, (PB // 2, 128), 1)
        for c in range(NQ):
            o, t = (80 * c) % 128, (80 * c) // 128
            tile = kb[:, t * 128:(t + 1) * 128]
            if o + 80 > 128:
                tile = jnp.where(lane_k >= o, tile, kb[:, (t + 1) * 128:(t + 2) * 128])
            if o:
                tile = pltpu.roll(tile, 128 - o, 1)
            k4_v[pl.ds(pl.multiple_of(j * (PB // 2), PB // 2), PB // 2), c * 128:(c + 1) * 128] = tile

        rowq = lax.broadcasted_iota(i32, (40, 128), 0)
        odd = jnp.broadcast_to((rowq >= 20)[None], (H // 2, 40, 128)).reshape(D, 128)
        for t in range(PB // 128):
            tt = j * (PB // 128) + t
            xb = x_v[pl.ds(pl.multiple_of(tt * 128, 128), 128), :]
            qv = lax.dot_general(wqvT_v[...], xb, (((1,), (1,)), ((), ())),
                                 preferred_element_type=f32)
            q = qv[:D] * QSCALE
            q = jnp.where(odd, pltpu.roll(q, 64, 1), q)
            qm_v[:, pl.ds(pl.multiple_of(tt * 128, 128), 128)] = _bc32(q.astype(bf16))
            v = jnp.concatenate([qv[D:].reshape(H // 2, 40, 128),
                                 jnp.ones((H // 2, 8, 128), f32)], axis=1)
            vt_v[tt] = _bc32(v.reshape(H // 2 * 48, 128).astype(bf16))

    def qv2(j, _):
        qv_proj(2 * j, None)
        qv_proj(2 * j + 1, None)

    lax.fori_loop(0, S // PB // 2, qv2, None)

    units = [(0, 0), (0, 1), (1, 0), (1, 1)]

    def qk_unit(c, T, i, r, nprev):
        lo = 16 * i
        qq = qm_v[pl.ds(pl.multiple_of(c * 40 + lo, 8), 24), pl.ds(pl.multiple_of(T * 128, 128), 128)]
        w = qq & mask_v[2 * i + r, lo:lo + 24]
        w = _bc16(jnp.concatenate(([jnp.zeros((lo, 128), i32)] if lo else [])
                                  + [w, jnp.zeros((64 - 24 - lo, 128), i32)], axis=0))
        if nprev == 2:
            krow, nrow = pl.multiple_of((T - 2) * 64 + 32 * r, 32), 160
        else:
            krow, nrow = 0, 64 * nprev + 32 * (r + 1)
        kk = _bc16(k4_v[pl.ds(krow, nrow), pl.ds(pl.multiple_of(c * 128, 128), 128)])
        return _dot(kk, w)

    def softmax_unit(s, r, nprev):
        n = s.shape[0]
        parts = []
        if nprev == 2:
            parts.append(s[0:64] + bias_v[0])
            parts.append(s[64:n - 64])
        elif n > 64:
            parts.append(s[0:n - 64])
        parts.append(s[n - 64:n] + bias_v[1])
        m8 = None
        for p in parts:
            pm = jnp.max(p.reshape(p.shape[0] // 8, 8, 128), axis=0)
            m8 = pm if m8 is None else jnp.maximum(m8, pm)
        m = jnp.max(m8, axis=0, keepdims=True)
        ps = [jnp.exp2(p - m) for p in parts]
        z = jnp.zeros((64, 128), f32)
        if r == 0:
            ps = ps + [z]
        elif nprev == 2:
            ps = [z] + ps
        return jnp.concatenate(ps, axis=0).astype(bf16)

    def pv_unit(c, T, i, pf, nprev):
        prow = pl.multiple_of((c * 2 + i) * 24, 8)
        vv = jnp.concatenate([_bc16(vt_v[T - nprev + j, pl.ds(prow, 24), :])
                              for j in range(nprev + 1)], axis=1)
        R = _dot(vv, pf)
        return (R[:40].reshape(5, 8, 128) * (1.0 / R[40:48])[None]).reshape(40, 128)

    def finish(c, T, Rs):
        lane_o = lax.broadcasted_iota(i32, (40, 128), 1)
        row_o = lax.broadcasted_iota(i32, (40, 128), 0)
        outs = []
        for i in range(2):
            R0, R1 = Rs[2 * i], Rs[2 * i + 1]
            A = jnp.where(lane_o < 64, R0, R1)
            B = pltpu.roll(jnp.where(lane_o < 64, R1, R0), 64, 1)
            outs.append(jnp.where(row_o < 20, A, B))
        o = jnp.concatenate(outs, axis=0).astype(bf16)
        ot_v[pl.ds(pl.multiple_of(c * 40, 8), 40), pl.ds(pl.multiple_of(T * 128, 128), 128)] = _bc32(o)

    def edge_slots(T, i, r):
        return 2 * i + (r if T == 0 else 1 - r), (0 if T == 0 else 64 * (2 - r))

    edge_units = [(T, i, r) for T in range(2) for (i, r) in units]

    def edge_qk(c, e, s_ref):
        T, i, r = edge_units[e]
        slot, r0 = edge_slots(T, i, r)
        s = qk_unit(c, T, i, r, T)
        s_ref[slot, r0:r0 + s.shape[0]] = s

    def edge_softmax(e, s_ref):
        T, i, r = edge_units[e]
        slot, r0 = edge_slots(T, i, r)
        return softmax_unit(s_ref[slot, r0:r0 + 64 * (2 * T + r + 1)], r, T)

    def ct(idx):
        return idx % NQ, idx // NQ + 2

    bufs = (sa_v, sb_v)
    for e in range(8):
        edge_qk(0, e, bufs[0])
    pend, Rs = [], {}

    def edge_pv():
        c, e, p = pend.pop(0)
        T, i, r = edge_units[e]
        Rs.setdefault((c, T), []).append(pv_unit(c, T, i, p, T))
        if e % 4 == 3:
            finish(c, T, Rs.pop((c, T)))

    for c in range(NQ):
        for e in range(8):
            if c + 1 < NQ:
                edge_qk(c + 1, e, bufs[(c + 1) % 2])
            elif e % 2 == 0:
                i, r = units[e // 2]
                bufs[(c + 1) % 2][e // 2] = qk_unit(0, 2, i, r, 2)
            pend.append((c, e, edge_softmax(e, bufs[c % 2])))
            if len(pend) > 2:
                edge_pv()
    while pend:
        edge_pv()

    ngroups = (NT - 2) * NQ
    NSTEP = 56

    def attn_body(it, _):
        LAG = 2
        pend, Rs = [], {}

        def do_pv():
            k, u, p = pend.pop(0)
            c, T = ct(NSTEP * it + k)
            Rs.setdefault(k, []).append(pv_unit(c, T, units[u][0], p, 2))
            if u == 3:
                finish(c, T, Rs.pop(k))

        for k in range(NSTEP):
            cur_ref, nxt_ref = bufs[k % 2], bufs[(k + 1) % 2]
            cn, Tn = ct(jnp.minimum(NSTEP * it + k + 1, ngroups - 1))
            for u, (i, r) in enumerate(units):
                nxt_ref[u] = qk_unit(cn, Tn, i, r, 2)
                pend.append((k, u, softmax_unit(cur_ref[u], r, 2)))
                if len(pend) > LAG:
                    do_pv()
        while pend:
            do_pv()

    lax.fori_loop(0, ngroups // NSTEP, attn_body, None)

    w1_copy.wait()
    w2_copy.wait()
    wo_copy.wait()
    gw_copy.wait()
    gw = gw_v[...].astype(f32).reshape(1, D)

    def out_copy(j, slot):
        return pltpu.make_async_copy(out_v.at[slot], out_hbm.at[pl.ds(pl.multiple_of(j * XB, XB), XB), :],
                                     osems.at[slot])

    def final(j, _):
        slot = j % 2
        t0 = pl.multiple_of(j * XB, XB)

        @pl.when(j >= 2)
        def _():
            out_copy(j - 2, slot).wait()

        xb = x_v[pl.ds(t0, XB), :]
        g = jax.nn.sigmoid(jnp.sum(xb.astype(f32) * gw, axis=1, keepdims=True))
        h = _dot(xb, w1_v[...])
        h = (h * jax.nn.sigmoid(h)).astype(bf16)
        b = _dot(h, w2_v[...])
        oT = _bc16(ot_v[:, pl.ds(t0, XB)])
        a = lax.dot_general(oT, wo_v[...], (((0,), (0,)), ((), ())), preferred_element_type=f32)
        out_v[slot] = (g * a + (1.0 - g) * b).astype(bf16)
        out_copy(j, slot).start()

    lax.fori_loop(0, nxb, final, None)
    out_copy(nxb - 2, 0).wait()
    out_copy(nxb - 1, 1).wait()


@jax.jit
def pallas_gated_mix__sliding_block__dense_activation_silu__prompt_kernel(
    A_x: jax.Array,
    A_wqkv: jax.Array,
    A_wo: jax.Array,
    B_x: jax.Array,
    B_w1: jax.Array,
    B_w2: jax.Array,
    gate_w: jax.Array,
):
    del B_x
    any_spec = pl.BlockSpec(memory_space=pl.ANY)
    out = pl.pallas_call(
        _kernel,
        out_shape=jax.ShapeDtypeStruct((S, D), bf16),
        in_specs=[any_spec] * 6,
        out_specs=any_spec,
        scratch_shapes=[
            pltpu.VMEM((S, D), bf16),
            pltpu.VMEM((D, 3 * D), bf16),
            pltpu.VMEM((D, D), bf16),
            pltpu.VMEM((D, F), bf16),
            pltpu.VMEM((F, D), bf16),
            pltpu.VMEM((D,), bf16),
            pltpu.VMEM((2 * D, D), bf16),
            pltpu.VMEM((S // 2, D), i32),
            pltpu.VMEM((D // 2, S), i32),
            pltpu.VMEM((S // 2, NQ * 128), i32),
            pltpu.VMEM((NT, H // 2 * 24, 128), i32),
            pltpu.VMEM((D // 2, S), i32),
            pltpu.VMEM((4, 40, 128), i32),
            pltpu.VMEM((2, 64, 128), f32),
            pltpu.VMEM((4, 320, 128), f32),
            pltpu.VMEM((4, 320, 128), f32),
            pltpu.VMEM((2, XB, D), bf16),
            pltpu.SemaphoreType.DMA((S // XB + 7,)),
            pltpu.SemaphoreType.DMA((2,)),
        ],
        compiler_params=pltpu.CompilerParams(vmem_limit_bytes=100 * 1024 * 1024),
    )(A_x.reshape(S, D), A_wqkv, A_wo, B_w1, B_w2, gate_w)
    return out.reshape(1, S, D)
```
